```python
import os as _os
_os.environ.setdefault("JAX_PLATFORMS", "cpu")
import jax
import jax.numpy as jnp

def _softmax(x, axis=-1):
    return jax.nn.softmax(x, axis=axis)
def _gelu(x):
    return jax.nn.gelu(x, approximate=True)
def _silu(x):
    return jax.nn.silu(x)
def _sigmoid(x):
    return jax.nn.sigmoid(x)
def _layernorm(x, axis=-1, eps=1e-5):
    m = jnp.mean(x, axis=axis, keepdims=True)
    v = jnp.var(x, axis=axis, keepdims=True)
    return (x - m) / jnp.sqrt(v + eps)
def _scatter_add(tgt, idx, src, axis=0):
    return tgt.at[idx].add(src)
def _segment_sum(src, seg, n):
    return jax.ops.segment_sum(src, seg, n)
class _Rng:
    def __init__(self, key):
        self._k = key
    def _next(self):
        self._k, sub = jax.random.split(self._k)
        return sub
    def normal(self, shape):
        return jax.random.normal(self._next(), shape, dtype=jnp.bfloat16)
    def randint(self, lo, hi, shape):
        return jax.random.randint(self._next(), shape, lo, hi, dtype=jnp.int32)
    def uniform(self, shape, lo=0.0, hi=1.0):
        return jax.random.uniform(self._next(), shape, jnp.bfloat16, lo, hi)
    def permutation(self, n):
        return jax.random.permutation(self._next(), n)


kernel_name = 'concat_heads__gqa_block_cached__mha_block_cached__near_ridge'

def setup_inputs():
    _rng = _Rng(jax.random.key(int.from_bytes(__import__("os").urandom(4), "little")))
    _w = (lambda a: (lambda t: t.astype(jnp.bfloat16) if jnp.issubdtype(t.dtype, jnp.floating) else t)(jnp.asarray(a)))
    def _A_setup():
        B, Sq, D = 8, 48, 512
        Hq, Hkv, Sk, Dh = 32, 8, 1024, 128
        assert Hq % Hkv == 0, (Hq, Hkv)
        return {
            "x": _w((lambda *s: _rng.normal(s) * 0.8)(B, Sq, D)),
            "k_cache": _w((lambda *s: _rng.normal(s) * 0.8)(B, Hkv, Sk, Dh)),
            "v_cache": _w((lambda *s: _rng.normal(s) * 0.05)(B, Hkv, Sk, Dh)),
            "wq": _w((lambda *s: _rng.normal(s) * 0.8)(D, Hq * Dh) * (D ** -0.5)),
            "wo": _w((lambda *s: _rng.normal(s) * 0.05)(Hq * Dh, D) * ((Hq * Dh) ** -0.5)),
        }
    _A_in = _A_setup()

    def _B_setup():
        B, Sq, D = 8, 48, 512
        H, Sk, Dh = 32, 1024, 128
        return {
            "x": _w((lambda *s: _rng.normal(s) * 0.8)(B, Sq, D)),
            "k_cache": _w((lambda *s: _rng.normal(s) * 0.8)(B, H, Sk, Dh)),
            "v_cache": _w((lambda *s: _rng.normal(s) * 0.05)(B, H, Sk, Dh)),
            "wq": _w((lambda *s: _rng.normal(s) * 0.8)(D, H * Dh) * (D ** -0.5)),
            "wo": _w((lambda *s: _rng.normal(s) * 0.05)(H * Dh, D) * ((H * Dh) ** -0.5)),
        }
    _B_in = _B_setup()

    return {
        "A_x": _A_in["x"],
        "A_k_cache": _A_in["k_cache"],
        "A_v_cache": _A_in["v_cache"],
        "A_wq": _A_in["wq"],
        "A_wo": _A_in["wo"],
        "B_x": _B_in["x"],
        "B_k_cache": _B_in["k_cache"],
        "B_v_cache": _B_in["v_cache"],
        "B_wq": _B_in["wq"],
        "B_wo": _B_in["wo"],
    }

def reference(A_x, A_k_cache, A_v_cache, A_wq, A_wo, B_x, B_k_cache, B_v_cache, B_wq, B_wo):
    def _A_ref(x, k_cache, v_cache, wq, wo):
        B, Sq, D = x.shape
        Hq, Dh = 32, 128
        Hkv = k_cache.shape[1]
        rep = Hq // Hkv
        q = (lambda x, *d: x.transpose(*d))((x @ wq).reshape(B, Sq, Hq, Dh), 0, 2, 1, 3)
        k = jnp.repeat(k_cache, rep, axis=1)
        v = jnp.repeat(v_cache, rep, axis=1)
        scores = jnp.einsum("bhqd,bhkd->bhqk", q, k) * (Dh ** -0.5)
        p = _softmax(scores, axis=-1)
        o = jnp.einsum("bhqk,bhkd->bhqd", p, v)
        return (lambda x, *d: x.transpose(*d))(o, 0, 2, 1, 3).reshape(B, Sq, Hq * Dh) @ wo

    def _B_ref(x, k_cache, v_cache, wq, wo):
        B, Sq, D = x.shape
        H, Dh = 32, 128
        q = (lambda x, *d: x.transpose(*d))((x @ wq).reshape(B, Sq, H, Dh), 0, 2, 1, 3)
        scores = jnp.einsum("bhqd,bhkd->bhqk", q, k_cache) * (Dh ** -0.5)
        p = _softmax(scores, axis=-1)
        o = jnp.einsum("bhqk,bhkd->bhqd", p, v_cache)
        return (lambda x, *d: x.transpose(*d))(o, 0, 2, 1, 3).reshape(B, Sq, H * Dh) @ wo

    a = _A_ref(A_x, A_k_cache, A_v_cache, A_wq, A_wo)
    b = _B_ref(B_x, B_k_cache, B_v_cache, B_wq, B_wo)
    return jnp.concatenate([a, b], axis=-1)
```

```python
import math
import jax
import jax.numpy as jnp
from jax import lax
from jax.experimental import pallas as pl
from jax.experimental.pallas import tpu as pltpu

NB, SQ, D = 8, 48, 512
HQ, HKV, SK, DH = 32, 8, 1024, 128
NIT = 64
QSCALE = (DH ** -0.5) * math.log2(math.e)
F32, BF16 = jnp.float32, jnp.bfloat16


def make(do_compute=True, do_dma=True, rows=128, nslot=3, pace="pair", k_prio=0, qk_split=2, pv_split=2,
         flags=None, stream_order="BBBBA", n_paced=14, u32=False):
    nchunk = SK // rows

    def kern(xa_hbm, ka_hbm, va_hbm, wqa_hbm, woa_hbm, xb_hbm, kb_hbm, vb_hbm, wqb_hbm, wob_hbm, out_hbm,
             xa, xb, wqa, wqb, woa, wob, kbuf, vbuf, acca, accb, obuf, ksem, vsem, wsem, xsem, osem):

        def kv_pairs(i, slot):
            j = i // 2
            b0 = (i % 2) * 4
            g = i // 8
            ba = i % 8
            pairs = []
            for c in range(nchunk):
                r = pl.ds(c * rows, rows)
                u = 0
                for ch in stream_order:
                    if ch == "B":
                        pairs.append((
                            lambda u=u, r=r: pltpu.make_async_copy(kb_hbm.at[b0 + u, j, r], kbuf.at[slot, u, r], ksem.at[slot]),
                            lambda u=u, r=r: pltpu.make_async_copy(vb_hbm.at[b0 + u, j, r], vbuf.at[slot, u, r], vsem.at[slot])))
                        u += 1
                    else:
                        pairs.append((
                            lambda r=r: pltpu.make_async_copy(ka_hbm.at[ba, g, r], kbuf.at[slot, 4, r], ksem.at[slot]),
                            lambda r=r: pltpu.make_async_copy(va_hbm.at[ba, g, r], vbuf.at[slot, 4, r], vsem.at[slot])))
            return pairs

        def w_pairs(grp, part, slot):
            pairs = []
            cols = pl.ds(pl.multiple_of(grp * 512, 512), 512)
            for half in range(2):
                r = pl.ds(pl.multiple_of(part * 64 + half * 32, 32), 32)
                ro = pl.ds(pl.multiple_of(grp * 512 + part * 64 + half * 32, 32), 32)
                pairs.append((
                    lambda r=r: pltpu.make_async_copy(wqa_hbm.at[r, cols], wqa.at[grp, r], ksem.at[slot]),
                    lambda r=r, ro=ro: pltpu.make_async_copy(woa_hbm.at[ro], woa.at[grp, r], vsem.at[slot])))
                pairs.append((
                    lambda r=r: pltpu.make_async_copy(wqb_hbm.at[r, cols], wqb.at[grp, r], ksem.at[slot]),
                    lambda r=r, ro=ro: pltpu.make_async_copy(wob_hbm.at[ro], wob.at[grp, r], vsem.at[slot])))
            return pairs

        def merge(kv, w):
            out = []
            step = len(kv) / len(w)
            nxt = step / 2
            wi = 0
            for n, p in enumerate(kv):
                out.append(p)
                if n + 1 >= nxt and wi < len(w):
                    out.append(w[wi])
                    wi += 1
                    nxt += step
            out += w[wi:]
            return out

        def pairs_for(i, slot, with_w=True):
            kv = kv_pairs(i, slot)
            if not with_w:
                return kv
            return merge(kv, w_pairs((i + 7) // 8, (i + 7) % 8, slot))

        def start_pair(p):
            if do_dma:
                p[1]().start(priority=1 - k_prio)
                p[0]().start(priority=k_prio)

        def wait_pair(p):
            if do_dma:
                if k_prio == 0:
                    p[1]().wait()
                    p[0]().wait()
                else:
                    p[0]().wait()
                    p[1]().wait()

        def compute_pieces(i, slot):
            j = i // 2
            half = i % 2
            g = i // 8
            ba = i % 8
            hh = j % 4
            st = {}
            pieces = []

            def qproj_b():
                x = jnp.concatenate([ld(xb, half * 4 + t, (0, SQ), slice(None)) for t in range(4)], axis=0)
                w = ld(wqb, g, (0, D), pl.ds(pl.multiple_of(hh * DH, DH), DH))
                q = jnp.dot(x, w, preferred_element_type=F32) * QSCALE
                st["qb"] = [q[u * SQ:(u + 1) * SQ].astype(BF16) for u in range(4)]
            pieces.append(qproj_b)

            def qproj_a():
                q = jnp.dot(ld(xa, ba, (0, SQ), slice(None)), ld(wqa, g, (0, D), slice(None)), preferred_element_type=F32) * QSCALE
                st["qa"] = jnp.concatenate([q[:, h * DH:(h + 1) * DH] for h in range(4)], axis=0).astype(BF16)
            pieces.append(qproj_a)

            def add_unit(u):
                kc = SK // qk_split
                vc = SK // pv_split
                for c in range(qk_split):
                    def qk(c=c):
                        q = st["qb"][u] if u < 4 else st["qa"]
                        k = ld(kbuf, slot, u, (c * kc, kc), slice(None))
                        st[("s", u, c)] = lax.dot_general(q, k, (((1,), (1,)), ((), ())), preferred_element_type=F32)
                    pieces.append(qk)

                def smax():
                    s = jnp.concatenate([st[("s", u, c)] for c in range(qk_split)], axis=1)
                    m = jnp.max(s, axis=-1, keepdims=True)
                    p = jnp.exp2(s - m)
                    st[("l", u)] = jnp.sum(p, axis=-1, keepdims=True)
                    st[("p", u)] = [p[:, c * vc:(c + 1) * vc].astype(BF16) for c in range(pv_split)]
                pieces.append(smax)
                for c in range(pv_split):
                    def pv(c=c):
                        v = ld(vbuf, slot, u, (c * vc, vc), slice(None))
                        o = jnp.dot(st[("p", u)][c], v, preferred_element_type=F32)
                        st[("o", u)] = o if c == 0 else st[("o", u)] + o
                        if c == pv_split - 1:
                            st[("o", u)] = st[("o", u)] * (1.0 / st[("l", u)])
                    pieces.append(pv)

            for u in range(4):
                add_unit(u)

            def oproj_b():
                o = jnp.concatenate([st[("o", u)] for u in range(4)], axis=0).astype(BF16)
                w = ld(wob, g, (pl.multiple_of(hh * DH, DH), DH), slice(None))
                r = pl.ds(pl.multiple_of(half * 4 * SQ, 4 * SQ), 4 * SQ)
                accb[r, :] += jnp.dot(o, w, preferred_element_type=F32)
            pieces.append(oproj_b)

            add_unit(4)

            def oproj_a():
                o = st[("o", 4)]
                o = jnp.concatenate([o[h * SQ:(h + 1) * SQ] for h in range(4)], axis=1).astype(BF16)
                r = pl.ds(pl.multiple_of(ba * SQ, SQ), SQ)
                acca[r, :] += jnp.dot(o, ld(woa, g, (0, 512), slice(None)), preferred_element_type=F32)
            pieces.append(oproj_a)
            return pieces

        def run_iteration(i, slot, waits, starts):
            pieces = compute_pieces(i, slot) if do_compute else []
            n = len(pieces)
            n2 = max(len(starts) - n_paced, 0) if do_compute else 0
            done = 0
            for pt in range(n2):
                start_pair(starts[pt])
                upto = ((pt + 1) * n) // n2
                while done < upto:
                    pieces[done]()
                    done += 1
            while done < n:
                pieces[done]()
                done += 1
            nw0 = len(waits) - (len(starts) - n2)
            for pt in range(nw0):
                wait_pair(waits[pt])
            for pt in range(len(starts) - n2):
                wait_pair(waits[nw0 + pt])
                start_pair(starts[n2 + pt])

        def ld(ref, *idx):
            lead = idx[:-2]
            (r0, nr), c = idx[-2], idx[-1]
            if not u32:
                return ref[(*lead, pl.ds(r0, nr), c)]
            r0 = r0 // 2 if isinstance(r0, int) else pl.multiple_of(r0 // 2, 8)
            return pltpu.bitcast(ref.bitcast(jnp.uint32)[(*lead, pl.ds(r0, nr // 2), c)], BF16)

        cxa = pltpu.make_async_copy(xa_hbm, xa, xsem.at[0])
        cxb = pltpu.make_async_copy(xb_hbm, xb, xsem.at[1])
        w0 = []
        for part in range(8):
            w0 += w_pairs(0, part, 0)
        first = merge(kv_pairs(0, 0), w0)
        second = pairs_for(1, 1)
        depth = len(second)
        cxa.start(priority=1)
        cxb.start(priority=0)
        stream = first + second
        for p in stream[:depth]:
            start_pair(p)
        acca[...] = jnp.zeros_like(acca)
        accb[...] = jnp.zeros_like(accb)
        cxa.wait()
        cxb.wait()
        for n, p in enumerate(first):
            wait_pair(p)
            start_pair(stream[depth + n])

        def body_w(i, slot):
            s1 = jnp.where(slot + 1 >= nslot, slot + 1 - nslot, slot + 1)
            s2 = jnp.where(slot + 2 >= nslot, slot + 2 - nslot, slot + 2)
            run_iteration(i, slot, pairs_for(i + 1, s1), pairs_for(i + 2, s2))
            return s1

        def body_now(i, slot):
            s1 = jnp.where(slot + 1 >= nslot, slot + 1 - nslot, slot + 1)
            s2 = jnp.where(slot + 2 >= nslot, slot + 2 - nslot, slot + 2)
            run_iteration(i, slot, pairs_for(i + 1, s1, False), pairs_for(i + 2, s2, False))
            return s1

        lax.fori_loop(0, 55, body_w, 0)
        run_iteration(55, 55 % nslot, pairs_for(56, 56 % nslot), pairs_for(57, 57 % nslot, False))
        lax.fori_loop(56, 62, body_now, 56 % nslot)
        run_iteration(62, 62 % nslot, pairs_for(63, 63 % nslot, False), [])
        run_iteration(63, 63 % nslot, [], [])

        obuf[:, :, :D] = acca[...].astype(BF16).reshape(NB, SQ, D)
        obuf[:, :, D:] = accb[...].astype(BF16).reshape(NB, SQ, D)
        co = pltpu.make_async_copy(obuf, out_hbm, osem)
        co.start()
        co.wait()

    def fn(A_x, A_k_cache, A_v_cache, A_wq, A_wo, B_x, B_k_cache, B_v_cache, B_wq, B_wo):
        any_spec = pl.BlockSpec(memory_space=pl.ANY)
        return pl.pallas_call(
            kern,
            in_specs=[any_spec] * 10,
            out_specs=any_spec,
            out_shape=jax.ShapeDtypeStruct((NB, SQ, 2 * D), BF16),
            scratch_shapes=[
                pltpu.VMEM((NB, SQ, D), BF16), pltpu.VMEM((NB, SQ, D), BF16),
                pltpu.VMEM((8, D, 512), BF16), pltpu.VMEM((8, D, 512), BF16),
                pltpu.VMEM((8, 512, D), BF16), pltpu.VMEM((8, 512, D), BF16),
                pltpu.VMEM((nslot, 5, SK, DH), BF16), pltpu.VMEM((nslot, 5, SK, DH), BF16),
                pltpu.VMEM((NB * SQ, D), F32), pltpu.VMEM((NB * SQ, D), F32),
                pltpu.VMEM((NB, SQ, 2 * D), BF16),
                pltpu.SemaphoreType.DMA((nslot,)), pltpu.SemaphoreType.DMA((nslot,)),
                pltpu.SemaphoreType.DMA((2,)), pltpu.SemaphoreType.DMA((2,)), pltpu.SemaphoreType.DMA(()),
            ],
            compiler_params=pltpu.CompilerParams(
                vmem_limit_bytes=100 * 1024 * 1024, disable_bounds_checks=True, flags=flags),
            name="fused_attn",
        )(A_x, A_k_cache, A_v_cache, A_wq, A_wo, B_x, B_k_cache, B_v_cache, B_wq, B_wo)

    return fn


@jax.jit
def pallas_concat_heads__gqa_block_cached__mha_block_cached__near_ridge_kernel(
    A_x, A_k_cache, A_v_cache, A_wq, A_wo, B_x, B_k_cache, B_v_cache, B_wq, B_wo,
):
    return make()(A_x, A_k_cache, A_v_cache, A_wq, A_wo, B_x, B_k_cache, B_v_cache, B_wq, B_wo)
```

```python
import contextlib
import math
import jax
import jax.numpy as jnp
from jax import lax
from jax.experimental import pallas as pl
from jax.experimental.pallas import tpu as pltpu

NB, SQ, D = 8, 48, 512
HQ, HKV, SK, DH = 32, 8, 1024, 128
NIT = 64
PG = 128
NPG = SK // PG
QSCALE = (DH ** -0.5) * math.log2(math.e)
F32, BF16 = jnp.float32, jnp.bfloat16
NT = (((1,), (1,)), ((), ()))


def mult(x, n):
    return x if isinstance(x, int) else pl.multiple_of(x, n)


def make(do_compute=True, do_dma=True, lk=18, lv=50, split=1, flags=None, sem_checks=False,
         piece_order="qa,qb,K4,K0,S4,K1,S0,V4,K2,S1,V0,K3,S2,V1,oa,S3,V2,V3,ob",
         tail_order="K0,K1,S0,K2,S1,V0,K3,S2,V1,qn,S3,V2,V3,ob",
         nslot=4, scopes=False, stream_order="BBABB", tail_compute=True, batches=None,
         out_mode="split", bulk_left=8, wprio=(0, 0, 0), k_keep=None, k_parts=8, ahead=2,
         wlead=16, vshift=0, bmap="half", amap=0, span=1.0, tail_split=1, last_hi=0):
    scope = jax.named_scope if scopes else (lambda n: contextlib.nullcontext())
    k_keep = lk if k_keep is None else k_keep

    def kern(xa_hbm, ka_hbm, va_hbm, wqa_hbm, woa_hbm, xb_hbm, kb_hbm, vb_hbm, wqb_hbm, wob_hbm, out_hbm,
             xa, xb, wqa, wqb, woa, wob, kbuf, vbuf, acca, accb, obuf, sems, wsem, osem):

        def start(c, prio):
            if do_dma:
                c.start(priority=prio)

        def wait(c):
            if do_dma:
                c.wait()

        LAST = NIT + ahead - 1
        stream = []
        for c in range(NPG):
            u = 0
            for ch in stream_order:
                if ch == "B":
                    stream.append((u, c))
                    u += 1
                elif ch == "A":
                    stream.append((4, c))
                else:
                    stream.append((int(ch), c))
        npage = len(stream)
        streams = {"k": stream, "v": [(u, (c + vshift) % NPG) for u, c in stream]}

        def a_batch(s):
            return (s + amap) % 8

        def sem_of(kind, is_a, slot):
            return sems.at[slot * 4 + (2 if is_a else 0) + (1 if kind == "v" else 0)]

        def page(kind, s, slot, n):
            u, c = streams[kind][n]
            r = pl.ds(c * PG, PG)
            dst = (kbuf if kind == "k" else vbuf).at[slot, u, r]
            if u == 4:
                src = (ka_hbm if kind == "k" else va_hbm).at[a_batch(s), s // 8, r]
            else:
                g = s - ahead
                src = (kb_hbm if kind == "k" else vb_hbm).at[(g % 2) * 4 + u, g // 2, r]
            return pltpu.make_async_copy(src, dst, sem_of(kind, u == 4, slot))

        b_pages = [n for n in range(npage) if stream[n][0] < 4]
        v_late = b_pages[len(b_pages) - last_hi:] if last_hi else []

        def start_page(kind, s, slot, n):
            prio = 0 if kind == "k" else 1
            static = isinstance(s, int)
            when = (lambda cond, fn: fn() if cond else None) if static else (lambda cond, fn: pl.when(cond)(fn))
            both = (lambda a, b: a and b) if static else jnp.logical_and
            last = LAST - 1 if ((kind == "k" and n >= k_keep) or (kind == "v" and n in v_late)) else LAST
            cond = s < NIT if stream[n][0] == 4 else both(s >= ahead, s <= last)
            when(cond, lambda: start(page(kind, s, slot, n), prio))

        def wait_part(kind, is_a, slot):
            buf = kbuf if kind == "k" else vbuf
            dst = buf.at[slot, 4] if is_a else buf.at[slot, pl.ds(0, 4)]
            wait(pltpu.make_async_copy(dst, dst, sem_of(kind, is_a, slot)))

        def q_proj_b(grp):
            x = xb[pl.ds(mult((grp % 2) * 4 * SQ, 4 * SQ), 4 * SQ), :]
            w = wqb[:, pl.ds(mult((grp // 2) * DH, DH), DH)]
            q = jnp.dot(x, w, preferred_element_type=F32) * QSCALE
            return [q[u * SQ:(u + 1) * SQ].astype(BF16) for u in range(4)]

        def compute_pieces(a, grp, slot, order, st, nsplit, final=False):
            groups = {}
            kc = SK // nsplit

            def qproj_b():
                st["qb"] = q_proj_b(grp)
            groups["qb"] = [qproj_b]

            def qproj_next():
                st["qn"] = q_proj_b(grp + 1)
            groups["qn"] = [qproj_next]

            def qproj_a():
                w = wqa[:, pl.ds(mult((a // 8) * 512, 512), 512)]
                q = jnp.dot(xa[pl.ds(mult(a_batch(a) * SQ, SQ), SQ), :], w, preferred_element_type=F32) * QSCALE
                st["qa"] = jnp.concatenate([q[:, h * DH:(h + 1) * DH] for h in range(4)], axis=0).astype(BF16)
            groups["qa"] = [qproj_a]

            for u in range(5):
                def qk(c, u=u):
                    q = st["qb"][u] if u < 4 else st["qa"]
                    k = kbuf[slot, u, pl.ds(c * kc, kc), :]
                    st[("s", u, c)] = lax.dot_general(q, k, NT, preferred_element_type=F32)

                def smax(u=u):
                    s = jnp.concatenate([st[("s", u, c)] for c in range(nsplit)], axis=1)
                    m = jnp.max(s, axis=-1, keepdims=True)
                    p = jnp.exp2(s - m)
                    st[("l", u)] = 1.0 / jnp.sum(p, axis=-1, keepdims=True)
                    st[("p", u)] = [p[:, c * kc:(c + 1) * kc].astype(BF16) for c in range(nsplit)]

                def pv(c, u=u):
                    v = vbuf[slot, u, pl.ds(c * kc, kc), :]
                    o = jnp.dot(st[("p", u)][c], v, preferred_element_type=F32)
                    st[("o", u)] = o if c == 0 else st[("o", u)] + o
                    if c == nsplit - 1:
                        st[("o", u)] = st[("o", u)] * st[("l", u)]

                groups["K%d" % u] = [lambda c=c, f=qk: f(c) for c in range(nsplit)]
                groups["S%d" % u] = [smax]
                groups["V%d" % u] = [lambda c=c, f=pv: f(c) for c in range(nsplit)]
                for c in range(nsplit):
                    groups["K%d%d" % (u, c)] = groups["K%d" % u][c:c + 1]
                    groups["V%d%d" % (u, c)] = groups["V%d" % u][c:c + 1]

            def oproj_b():
                o = jnp.concatenate([st[("o", u)] for u in range(4)], axis=0).astype(BF16)
                w = wob[pl.ds(mult((grp // 2) * DH, DH), DH), :]
                r = pl.ds(mult((grp % 2) * 4 * SQ, 4 * SQ), 4 * SQ)
                res = accb[r, :] + jnp.dot(o, w, preferred_element_type=F32)
                if final:
                    obuf[pl.ds((grp % 2) * 4, 4), :, pl.ds(D, D)] = res.astype(BF16).reshape(4, SQ, D)
                else:
                    accb[r, :] = res
            groups["ob"] = [oproj_b]

            def oproj_a():
                o = st[("o", 4)]
                o = jnp.concatenate([o[h * SQ:(h + 1) * SQ] for h in range(4)], axis=1).astype(BF16)
                w = woa[pl.ds(mult((a // 8) * 512, 512), 512), :]
                r = pl.ds(mult(a_batch(a) * SQ, SQ), SQ)
                res = acca[r, :] + jnp.dot(o, w, preferred_element_type=F32)
                acca[r, :] = res
                obuf[a_batch(a), :, pl.ds(0, D)] = res.astype(BF16)
            groups["oa"] = [oproj_a]
            return [p for name in order.split(",") for p in groups[name]]

        def interleave(pieces, starts, pos):
            done = 0
            for at, f in zip(pos, starts):
                while done < min(at, len(pieces)):
                    pieces[done]()
                    done += 1
                f()
            for p in pieces[done:]:
                p()

        def wq_page(which, pg):
            h, v = ((wqa_hbm, wqa), (wqb_hbm, wqb))[which]
            idx = (pl.ds(mult((pg // 2) * 8, 8), 8), pl.ds(mult((pg % 2) * 2048, 2048), 2048))
            return pltpu.make_async_copy(h.at[idx], v.at[idx], wsem.at[which])

        def wo_page(which, pg, late):
            h, v = ((woa_hbm, woa), (wob_hbm, wob))[which]
            r = pl.ds(mult(pg * 32, 32), 32)
            return pltpu.make_async_copy(h.at[r], v.at[r], wsem.at[2 + 2 * late + which])

        def x_page(which, pg):
            h, v = ((xa_hbm, xa), (xb_hbm, xb))[which]
            r = pl.ds(pg * 32, 32)
            return pltpu.make_async_copy(h.at[r], v.at[r], wsem.at[6 + which])

        a_pages = [n for n in range(npage) if stream[n][0] == 4]
        lo_q = [x_page(0, pg) for pg in range(12)] + [page("v", s, s, n) for s in range(ahead) for n in a_pages]
        hi_q = [x_page(1, pg) for pg in range(12)] + [page("k", s, s, n) for s in range(ahead) for n in a_pages
                                                      if s == 0 or n < lk]
        for n in range(len(lo_q) + wlead):
            if n < len(lo_q):
                start(lo_q[n], 1)
            if 0 <= n - wlead < len(hi_q):
                start(hi_q[n - wlead], 0)

        def early_body(t, carry):
            for reg in range(2):
                pg = reg * 32 + t
                start(wo_page(0, pg, 0), 1)
                start(wq_page(0, pg, ), 0)
                start(wo_page(1, pg, 0), 1)
                start(wq_page(1, pg), 0)
                start(wq_page(0, 64 + pg), 1)
                start(wq_page(1, 64 + pg), 0)

            @pl.when(t >= 16)
            def _():
                z = t - 16
                ra = pl.ds(pl.multiple_of(z * 24, 8), 24)
                acca[ra, :] = jnp.zeros((24, D), F32)
                accb[ra, :] = jnp.zeros((24, D), F32)
                rk = pl.ds(pl.multiple_of((z % 4) * 256, 256), 256)
                for sl in range(ahead):
                    kbuf[sl, z // 4, rk, :] = jnp.zeros((256, DH), BF16)
                    vbuf[sl, z // 4, rk, :] = jnp.zeros((256, DH), BF16)
            return carry

        def late_body(t, carry):
            for reg in range(4):
                pg = 64 + reg * 16 + t
                start(wo_page(0, pg, 1), 1)
                start(wo_page(1, pg, 1), 0)
            return carry

        with scope("wloop"):
            lax.fori_loop(0, 32, early_body, 0)
            lax.fori_loop(0, 12, late_body, 0)
        lo_q = [wo_page(0, 64 + reg * 16 + t, 1) for t in range(12, 16) for reg in range(4)]
        hi_q = [wo_page(1, 64 + reg * 16 + t, 1) for t in range(12, 16) for reg in range(4)]
        v_first = [page("v", p // npage, (p // npage) % nslot, p % npage) for p in range(ahead * npage, npage + lv)]
        k_first = [page("k", p // npage, (p // npage) % nslot, p % npage) for p in range(ahead * npage, npage + lk)]
        move = (len(v_first) - len(k_first)) // 2
        hi_q = hi_q + lo_q[:move] + k_first
        lo_q = lo_q[move:] + v_first
        for n in range(max(len(lo_q), len(hi_q))):
            if n < len(lo_q):
                start(lo_q[n], 1)
            if n < len(hi_q):
                start(hi_q[n], 0)
        with scope("wait0"):
            for buf, n in ((xa, 6), (xb, 7), (wqa, 0), (wqb, 1)):
                wait(pltpu.make_async_copy(buf, buf, wsem.at[n]))
            for n, buf in enumerate((woa, wob)):
                half = buf.at[pl.ds(0, 2048)]
                wait(pltpu.make_async_copy(half, half, wsem.at[2 + n]))
            wait_part("k", True, 0)
            wait_part("v", True, 0)

        def body(i, slot):
            def start_at(kind, off):
                ds, n = divmod(off, npage)
                start_page(kind, i + 1 + ds, (slot + 1 + ds) % nslot, n)

            def start_pair(pt):
                start_at("v", lv + pt)
                start_at("k", lk + pt)

            pieces = compute_pieces(i, jnp.maximum(i - ahead, 0), slot, piece_order, {}, split) if do_compute else []
            if batches is None or not do_compute:
                pos = [int(pt * len(pieces) * span) // npage for pt in range(npage)]
            else:
                pos = [at for at, cnt in batches for _ in range(cnt)]
            assert len(pos) == npage
            interleave(pieces, [lambda pt=pt: start_pair(pt) for pt in range(npage)], pos)
            s1 = (slot + 1) % nslot

            @pl.when(i == 1)
            def _():
                for n, buf in enumerate((woa, wob)):
                    half = buf.at[pl.ds(2048, 2048)]
                    wait(pltpu.make_async_copy(half, half, wsem.at[4 + n]))

            @pl.when(i + 1 < NIT)
            def _():
                wait_part("k", True, s1)
                wait_part("v", True, s1)

            @pl.when(i + 1 >= ahead)
            def _():
                wait_part("k", False, s1)
                wait_part("v", False, s1)
            return s1

        with scope("main"):
            tail_slot = lax.fori_loop(0, NIT, body, 0)

        assert ahead == 2 and (NIT + 1) * npage + lv >= (LAST + 1) * npage and k_keep <= lk
        k_rest = [n for n in range(k_keep, npage) if stream[n][0] < 4]

        def out_copy(b0, nb, c0, nc):
            idx = (pl.ds(b0, nb), slice(None), pl.ds(c0, nc))
            return pltpu.make_async_copy(obuf.at[idx], out_hbm.at[idx], osem)

        st = {}
        pieces = compute_pieces(0, NIT - 2, tail_slot, "qb," + tail_order, st, tail_split, True) if tail_compute else []
        starts = [lambda n=n: start(page("k", LAST, LAST % nslot, n), 0) for n in k_rest]
        interleave(pieces, starts, [(n * k_parts) // max(len(starts), 1) for n in range(len(starts))])
        with scope("waitk"):
            wait_part("k", False, LAST % nslot)
        st = {"qb": st.get("qn")}
        s1 = (tail_slot + 1) % nslot
        pieces = compute_pieces(0, NIT - 1, s1, "K0,K1,S0,K2,S1,K3,S2,S3", st, tail_split, True) if tail_compute else []
        starts = [lambda n=n: start(page("v", LAST, LAST % nslot, n), 0) for n in v_late]
        interleave(pieces, starts, [(n * len(pieces)) // max(len(starts), 1) for n in range(len(starts))])
        with scope("waitv"):
            for m, n in enumerate(b_pages):
                if m == len(b_pages) - bulk_left and out_mode == "split":
                    out_copy(0, 4, 0, 2 * D).start(priority=wprio[0])
                    out_copy(4, 4, 0, D).start(priority=wprio[1])
                wait(page("v", LAST, LAST % nslot, n))
        if tail_compute:
            interleave(compute_pieces(0, NIT - 1, s1, "V0,V1,V2,V3,ob", st, tail_split, True), [], [])
        out_copy(4, 4, D, D).start(priority=wprio[2])
        with scope("waitout"):
            if out_mode == "none":
                out_copy(4, 4, D, D).wait()
            else:
                pltpu.make_async_copy(obuf, obuf, osem).wait()

    def fn(A_x, A_k_cache, A_v_cache, A_wq, A_wo, B_x, B_k_cache, B_v_cache, B_wq, B_wo):
        any_spec = pl.BlockSpec(memory_space=pl.ANY)
        return pl.pallas_call(
            kern,
            in_specs=[any_spec] * 10,
            out_specs=any_spec,
            out_shape=jax.ShapeDtypeStruct((NB, SQ, 2 * D), BF16),
            scratch_shapes=[
                pltpu.VMEM((NB * SQ, D), BF16), pltpu.VMEM((NB * SQ, D), BF16),
                pltpu.VMEM((D, HQ * DH), BF16), pltpu.VMEM((D, HQ * DH), BF16),
                pltpu.VMEM((HQ * DH, D), BF16), pltpu.VMEM((HQ * DH, D), BF16),
                pltpu.VMEM((nslot, 5, SK, DH), BF16), pltpu.VMEM((nslot, 5, SK, DH), BF16),
                pltpu.VMEM((NB * SQ, D), F32), pltpu.VMEM((NB * SQ, D), F32),
                pltpu.VMEM((NB, SQ, 2 * D), BF16),
                pltpu.SemaphoreType.DMA((4 * nslot,)),
                pltpu.SemaphoreType.DMA((8,)), pltpu.SemaphoreType.DMA(()),
            ],
            compiler_params=pltpu.CompilerParams(
                vmem_limit_bytes=100 * 1024 * 1024, disable_bounds_checks=True,
                disable_semaphore_checks=not sem_checks, flags=flags),
            name="fused_attn",
        )(A_x.reshape(NB * SQ, D), A_k_cache, A_v_cache, A_wq, A_wo,
          B_x.reshape(NB * SQ, D), B_k_cache, B_v_cache, B_wq, B_wo)

    return fn


@jax.jit
def pallas_concat_heads__gqa_block_cached__mha_block_cached__near_ridge_kernel(
    A_x, A_k_cache, A_v_cache, A_wq, A_wo, B_x, B_k_cache, B_v_cache, B_wq, B_wo,
):
    return make()(A_x, A_k_cache, A_v_cache, A_wq, A_wo, B_x, B_k_cache, B_v_cache, B_wq, B_wo)
```

```python
import math

import jax
import jax.numpy as jnp
from jax import lax
import jax.experimental.pallas as pl
import jax.experimental.pallas.tpu as pltpu

BATCH, SEQ_Q, D_MODEL = 8, 48, 512
HEADS, HEAD_DIM, SEQ_K = 32, 128, 1024
GROUP = 4
STEPS = BATCH * HEADS // GROUP
AHEAD = 2
LAST_SET = STEPS + AHEAD - 1
A_UNIT = GROUP
SLOTS = 4

PAGE = 128
PAGES = SEQ_K // PAGE
UNIT_ORDER = (2, 1, 0, 3, A_UNIT)
K, V = 0, 1
PAGE_ORDER = (
    tuple((u, (c + 1) % PAGES) for c in range(PAGES) for u in UNIT_ORDER),
    tuple((u, c) for c in range(PAGES) for u in UNIT_ORDER),
)
SET_PAGES = len(PAGE_ORDER[K])
PRIORITY = (0, 1)
K_LOOK = 24
V_LOOK = K_LOOK + 32
LOOK = (K_LOOK, V_LOOK)
IN_COMPUTE = 20
V_SPLIT = 5 * PAGE
KB, VB_HEAD, VB_TAIL, KA, VA = range(5)

W_ROWS = 32
W_REGIONS, W_STEPS = 4, 32

Q_SCALE = HEAD_DIM ** -0.5 * math.log2(math.e)

HEAD_ORDER = "qa k4 s4 v4 oa"
MAIN_ORDER = "qa qb k4 k0 s4 k1 s0 v4 k2 s1 v0 k3 s2 v1 oa s3 v2 v3 ob"
TAIL_ORDER = "qb k0 k1 s0 k2 s1 v0 k3 s2 v1 qnext s3 v2 v3 ob"

F32, BF16 = jnp.float32, jnp.bfloat16


def _ds(index, size):
    start = index * size
    if not isinstance(start, int):
        start = pl.multiple_of(start, size)
    return pl.ds(start, size)


def _a_batch(unit):
    return (unit + BATCH - 1) % BATCH


def _b_head(group, u):
    g = group // BATCH
    return (g // GROUP) * GROUP * GROUP + g % GROUP + GROUP * u


def _interleave(stages, starts, first, last):
    done = 0
    for n, start in enumerate(starts):
        while done < first + (last - first) * n // len(starts):
            stages[done]()
            done += 1
        start()
    for stage in stages[done:]:
        stage()


def _kernel(xa_hbm, ka_hbm, va_hbm, wqa_hbm, woa_hbm,
            xb_hbm, kb_hbm, vb_hbm, wqb_hbm, wob_hbm, out_hbm,
            xa, xb, wqa, wqb, woa, wob, kv, acca, accb, out,
            kv_sem, w_sem, out_sem):

    def page(kind, s, slot, n):
        u, c = PAGE_ORDER[kind][n]
        rows = _ds(c, PAGE)
        if u == A_UNIT:
            src = (ka_hbm, va_hbm)[kind].at[_a_batch(s), s // BATCH, rows]
            sem = (KA, VA)[kind]
        else:
            group = s - AHEAD
            src = (kb_hbm, vb_hbm)[kind].at[group % BATCH, _b_head(group, u), rows]
            sem = KB if kind == K else (VB_HEAD if c * PAGE < V_SPLIT else VB_TAIL)
        return pltpu.make_async_copy(src, kv.at[slot, kind, u, rows], kv_sem.at[slot * 5 + sem])

    def wait_all(dst, sem):
        pltpu.make_async_copy(dst, dst, sem).wait()

    def wait_a(slot):
        wait_all(kv.at[slot, K, A_UNIT], kv_sem.at[slot * 5 + KA])
        wait_all(kv.at[slot, V, A_UNIT], kv_sem.at[slot * 5 + VA])

    def wait_b(slot, part):
        kind, r0, r1 = {KB: (K, 0, SEQ_K), VB_HEAD: (V, 0, V_SPLIT), VB_TAIL: (V, V_SPLIT, SEQ_K)}[part]
        wait_all(kv.at[slot, kind, pl.ds(0, GROUP), pl.ds(r0, r1 - r0)], kv_sem.at[slot * 5 + part])

    def start_pairs(low, high):
        extra = len(low) - len(high)
        for n, copy in enumerate(low):
            copy.start(priority=1)
            if n >= extra:
                high[n - extra].start(priority=0)

    def stages(order, unit, group, slot, val):
        def q_b(group):
            x = xb[_ds(group % BATCH, SEQ_Q), :]
            w = jnp.concatenate(
                [wqb[:, _ds(_b_head(group, u), HEAD_DIM)] for u in range(GROUP)], axis=1)
            q = jnp.dot(x, w, preferred_element_type=F32) * Q_SCALE
            return {u: q[:, u * HEAD_DIM:(u + 1) * HEAD_DIM].astype(BF16) for u in range(GROUP)}

        def q_a():
            x = xa[_ds(_a_batch(unit), SEQ_Q), :]
            w = wqa[:, _ds(unit // BATCH, GROUP * HEAD_DIM)]
            q = jnp.dot(x, w, preferred_element_type=F32) * Q_SCALE
            q = [q[:, h * HEAD_DIM:(h + 1) * HEAD_DIM] for h in range(GROUP)]
            return {A_UNIT: jnp.concatenate(q, axis=0).astype(BF16)}

        def scores(u):
            val["s", u] = lax.dot_general(val["q"][u], kv[slot, K, u], (((1,), (1,)), ((), ())),
                                          preferred_element_type=F32)

        def softmax(u):
            s = val["s", u]
            p = jnp.exp2(s - jnp.max(s, axis=-1, keepdims=True))
            val["inv", u] = 1.0 / jnp.sum(p, axis=-1, keepdims=True)
            val["p", u] = p.astype(BF16)

        def values(u, r0=0, r1=SEQ_K):
            o = jnp.dot(val["p", u][:, r0:r1], kv[slot, V, u, pl.ds(r0, r1 - r0), :],
                        preferred_element_type=F32)
            if r0 > 0:
                o = val["o", u] + o
            val["o", u] = o * val["inv", u] if r1 == SEQ_K else o

        def project(heads, w, acc, b, col):
            rows = _ds(b, SEQ_Q)
            o = jnp.concatenate(heads, axis=1).astype(BF16)
            res = acc[rows, :] + jnp.dot(o, w, preferred_element_type=F32)
            acc[rows, :] = res
            out[b, :, pl.ds(col, D_MODEL)] = res.astype(BF16)

        def out_a():
            o = val["o", A_UNIT]
            project([o[h * SEQ_Q:(h + 1) * SEQ_Q] for h in range(GROUP)],
                    woa[_ds(unit // BATCH, GROUP * HEAD_DIM), :], acca, _a_batch(unit), 0)

        def out_b():
            w = jnp.concatenate(
                [wob[_ds(_b_head(group, u), HEAD_DIM), :] for u in range(GROUP)], axis=0)
            project([val["o", u] for u in range(GROUP)], w, accb, group % BATCH, D_MODEL)

        table = {
            "qa": lambda: val["q"].update(q_a()),
            "qb": lambda: val["q"].update(q_b(group)),
            "qnext": lambda: val["qnext"].update(q_b(group + 1)),
            "oa": out_a,
            "ob": out_b,
        }
        for u in range(GROUP + 1):
            table[f"k{u}"] = lambda u=u: scores(u)
            table[f"s{u}"] = lambda u=u: softmax(u)
            table[f"v{u}"] = lambda u=u: values(u)
            table[f"head{u}"] = lambda u=u: values(u, 0, V_SPLIT)
            table[f"tail{u}"] = lambda u=u: values(u, V_SPLIT, SEQ_K)
        return [table[name] for name in order.split()]

    def run(order, unit, group, slot, val):
        for stage in stages(order, unit, group, slot, val):
            stage()

    def row_page(src, dst, n, sem):
        return pltpu.make_async_copy(src.at[_ds(n, W_ROWS)], dst.at[_ds(n, W_ROWS)], w_sem.at[sem])

    def wq_page(src, dst, n, sem):
        idx = (_ds(n // 2, 8), _ds(n % 2, HEADS * HEAD_DIM // 2))
        return pltpu.make_async_copy(src.at[idx], dst.at[idx], w_sem.at[sem])

    def a_pages(kind, s):
        return [page(kind, s, s, n) for n in range(SET_PAGES) if PAGE_ORDER[kind][n][0] == A_UNIT]

    def stream(kind, first, last):
        return [page(kind, p // SET_PAGES, p // SET_PAGES % SLOTS, p % SET_PAGES)
                for p in range(first, last)]

    for n in range(BATCH * SEQ_Q // W_ROWS):
        row_page(xa_hbm, xa, n, 4).start(priority=1)
        row_page(xb_hbm, xb, n, 5).start(priority=1)
    for copy in a_pages(V, 0):
        copy.start(priority=1)

    @pl.loop(0, W_STEPS)
    def _(t):
        for n in [region * W_STEPS + t for region in range(W_REGIONS)]:
            start_pairs([row_page(woa_hbm, woa, n, 2), wq_page(wqa_hbm, wqa, n, 0)],
                        [row_page(wob_hbm, wob, n, 3), wq_page(wqb_hbm, wqb, n, 1)])

    base = AHEAD * SET_PAGES
    start_pairs(stream(V, base, base + V_LOOK),
                a_pages(K, 0) + a_pages(K, 1) + a_pages(V, 1) + stream(K, base, base + K_LOOK))
    acca[...] = jnp.zeros_like(acca)
    accb[...] = jnp.zeros_like(accb)
    for n, buf in enumerate((wqa, wqb, woa, wob, xa, xb)):
        wait_all(buf, w_sem.at[n])
    wait_a(0)
    run(HEAD_ORDER, 0, None, 0, {"q": {}})
    wait_a(1)
    start_pairs(stream(V, base + V_LOOK, base + V_LOOK + SET_PAGES),
                stream(K, base + K_LOOK, base + K_LOOK + SET_PAGES))
    run(HEAD_ORDER, 1, None, 1, {"q": {}})
    wait_a(AHEAD)
    for part in (KB, VB_HEAD, VB_TAIL):
        wait_b(AHEAD, part)

    @pl.loop(AHEAD, STEPS)
    def _(i):
        def start(kind, n):
            skip, n = divmod(LOOK[kind] + n, SET_PAGES)
            s = i + 1 + skip
            end = STEPS if PAGE_ORDER[kind][n][0] == A_UNIT else LAST_SET + 1
            issue = lambda: page(kind, s, s % SLOTS, n).start(priority=PRIORITY[kind])
            if STEPS + skip < end:
                issue()
            else:
                pl.when(s < end)(issue)

        def start_pair(n):
            start(V, n)
            start(K, n)

        work = stages(MAIN_ORDER, i, i - AHEAD, i % SLOTS, {"q": {}})
        _interleave(work, [lambda n=n: start_pair(n) for n in range(IN_COMPUTE)], 2, len(work))

        @pl.when(i >= AHEAD)
        def _():
            for n in range(IN_COMPUTE, SET_PAGES):
                start_pair(n)

        slot = (i + 1) % SLOTS
        pl.when(i + 1 < STEPS)(lambda: wait_a(slot))
        for part in (KB, VB_HEAD, VB_TAIL):
            wait_b(slot, part)

    slot = LAST_SET % SLOTS
    b_pages = lambda kind: [n for n in range(SET_PAGES) if PAGE_ORDER[kind][n][0] != A_UNIT]
    val = {"q": {}, "qnext": {}}
    _interleave(stages(TAIL_ORDER, None, STEPS - 2, (LAST_SET - 1) % SLOTS, val),
                [lambda n=n: page(K, LAST_SET, slot, n).start(priority=PRIORITY[K])
                 for n in b_pages(K) if n >= K_LOOK], 0, 8)
    val = {"q": val["qnext"]}
    wait_b(slot, KB)
    run("k0 k1 s0 k2 s1 k3 s2 s3", None, STEPS - 1, slot, val)
    wait_b(slot, VB_HEAD)
    run("head0 head1 head2 head3", None, STEPS - 1, slot, val)

    def out_copy(b0, b1):
        rows = pl.ds(b0, b1 - b0)
        return pltpu.make_async_copy(out.at[rows], out_hbm.at[rows], out_sem)

    last_pages = [n for n in b_pages(V) if PAGE_ORDER[V][n][1] * PAGE >= V_SPLIT]
    for m, n in enumerate(last_pages):
        if m == 2:
            out_copy(0, BATCH - 1).start()
        page(V, LAST_SET, slot, n).wait()
    run("tail0 tail1 tail2 tail3 ob", None, STEPS - 1, slot, val)
    out_copy(BATCH - 1, BATCH).start()
    wait_all(out, out_sem)


@jax.jit
def pallas_concat_heads__gqa_block_cached__mha_block_cached__near_ridge_kernel(
    A_x: jax.Array,
    A_k_cache: jax.Array,
    A_v_cache: jax.Array,
    A_wq: jax.Array,
    A_wo: jax.Array,
    B_x: jax.Array,
    B_k_cache: jax.Array,
    B_v_cache: jax.Array,
    B_wq: jax.Array,
    B_wo: jax.Array,
):
    rows, inner = BATCH * SEQ_Q, HEADS * HEAD_DIM
    in_hbm = pl.BlockSpec(memory_space=pl.ANY)
    return pl.pallas_call(
        _kernel,
        in_specs=[in_hbm] * 10,
        out_specs=in_hbm,
        out_shape=jax.ShapeDtypeStruct((BATCH, SEQ_Q, 2 * D_MODEL), BF16),
        scratch_shapes=[
            pltpu.VMEM((rows, D_MODEL), BF16),
            pltpu.VMEM((rows, D_MODEL), BF16),
            pltpu.VMEM((D_MODEL, inner), BF16),
            pltpu.VMEM((D_MODEL, inner), BF16),
            pltpu.VMEM((inner, D_MODEL), BF16),
            pltpu.VMEM((inner, D_MODEL), BF16),
            pltpu.VMEM((SLOTS, 2, GROUP + 1, SEQ_K, HEAD_DIM), BF16),
            pltpu.VMEM((rows, D_MODEL), F32),
            pltpu.VMEM((rows, D_MODEL), F32),
            pltpu.VMEM((BATCH, SEQ_Q, 2 * D_MODEL), BF16),
            pltpu.SemaphoreType.DMA((5 * SLOTS,)),
            pltpu.SemaphoreType.DMA((6,)),
            pltpu.SemaphoreType.DMA(()),
        ],
        compiler_params=pltpu.CompilerParams(
            vmem_limit_bytes=64 * 1024 * 1024,
            disable_bounds_checks=True,
            disable_semaphore_checks=True,
        ),
        name="fused_attn",
    )(A_x.reshape(rows, D_MODEL), A_k_cache, A_v_cache, A_wq, A_wo,
      B_x.reshape(rows, D_MODEL), B_k_cache, B_v_cache, B_wq, B_wo)
```

```python
import math

import jax
import jax.numpy as jnp
from jax import lax
import jax.experimental.pallas as pl
import jax.experimental.pallas.tpu as pltpu

BATCH, SEQ_Q, D_MODEL = 8, 48, 512
HEADS, HEAD_DIM, SEQ_K = 32, 128, 1024
GROUP = 4
STEPS = BATCH * HEADS // GROUP
AHEAD = 2
LAST_SET = STEPS + AHEAD - 1
A_UNIT = GROUP
SLOTS = 4

PAGE = 128
PAGES = SEQ_K // PAGE
UNIT_ORDER = (3, 1, 0, 2, A_UNIT)
K, V = 0, 1
PAGE_ORDER = (
    tuple((u, (c + 1) % PAGES) for c in range(PAGES) for u in UNIT_ORDER),
    tuple((u, c) for c in range(PAGES) for u in UNIT_ORDER),
)
SET_PAGES = len(PAGE_ORDER[K])
PRIORITY = (0, 1)
K_LOOK = 24
V_LOOK = K_LOOK + 32
LOOK = (K_LOOK, V_LOOK)
IN_COMPUTE = 20
V_SPLIT = 5 * PAGE
WRITE_AT = (2, 10)
EARLY_BATCHES = 2
KB, VB_HEAD, VB_TAIL, KA, VA = range(5)

W_ROWS = 32
W_REGIONS, W_STEPS = 4, 32

Q_SCALE = HEAD_DIM ** -0.5 * math.log2(math.e)

HEAD_ORDER = "qa k4 s4 v4 oa"
MAIN_ORDER = "qa qb k4 k0 s4 k1 s0 v4 k2 s1 v0 k3 s2 v1 oa s3 v2 v3 ob"
TAIL_ORDER = "qb k0 k1 s0 k2 s1 v0 k3 s2 v1 qnext s3 v2 v3 ob"

F32, BF16 = jnp.float32, jnp.bfloat16


def _ds(index, size):
    start = index * size
    if not isinstance(start, int):
        start = pl.multiple_of(start, size)
    return pl.ds(start, size)


def _b_head(group, u):
    g = group // BATCH
    return (g // GROUP) * GROUP * GROUP + g % GROUP + GROUP * u


def _interleave(stages, starts, first, last):
    done = 0
    for n, start in enumerate(starts):
        while done < first + (last - first) * n // len(starts):
            stages[done]()
            done += 1
        start()
    for stage in stages[done:]:
        stage()


def _kernel(xa_hbm, ka_hbm, va_hbm, wqa_hbm, woa_hbm,
            xb_hbm, kb_hbm, vb_hbm, wqb_hbm, wob_hbm, out_hbm,
            xa, xb, wqa, wqb, woa, wob, kv, acca, accb, partial, out,
            kv_sem, w_sem, out_sem):

    def page(kind, s, slot, n):
        u, c = PAGE_ORDER[kind][n]
        rows = _ds(c, PAGE)
        if u == A_UNIT:
            src = (ka_hbm, va_hbm)[kind].at[s % BATCH, s // BATCH, rows]
            sem = (KA, VA)[kind]
        else:
            group = s - AHEAD
            src = (kb_hbm, vb_hbm)[kind].at[group % BATCH, _b_head(group, u), rows]
            sem = KB if kind == K else (VB_HEAD if c * PAGE < V_SPLIT else VB_TAIL)
        return pltpu.make_async_copy(src, kv.at[slot, kind, u, rows], kv_sem.at[slot * 5 + sem])

    def wait_all(dst, sem):
        pltpu.make_async_copy(dst, dst, sem).wait()

    def wait_a(slot):
        wait_all(kv.at[slot, K, A_UNIT], kv_sem.at[slot * 5 + KA])
        wait_all(kv.at[slot, V, A_UNIT], kv_sem.at[slot * 5 + VA])

    def wait_b(slot, part):
        kind, r0, r1 = {KB: (K, 0, SEQ_K), VB_HEAD: (V, 0, V_SPLIT), VB_TAIL: (V, V_SPLIT, SEQ_K)}[part]
        wait_all(kv.at[slot, kind, pl.ds(0, GROUP), pl.ds(r0, r1 - r0)], kv_sem.at[slot * 5 + part])

    def start_pairs(low, high):
        extra = len(low) - len(high)
        for n, copy in enumerate(low):
            copy.start(priority=1)
            if n >= extra:
                high[n - extra].start(priority=0)

    def stages(order, unit, group, slot, val):
        def q_b(group):
            x = xb[_ds(group % BATCH, SEQ_Q), :]
            w = jnp.concatenate(
                [wqb[:, _ds(_b_head(group, u), HEAD_DIM)] for u in range(GROUP)], axis=1)
            q = jnp.dot(x, w, preferred_element_type=F32) * Q_SCALE
            return {u: q[:, u * HEAD_DIM:(u + 1) * HEAD_DIM].astype(BF16) for u in range(GROUP)}

        def q_a():
            x = xa[_ds(unit % BATCH, SEQ_Q), :]
            w = wqa[:, _ds(unit // BATCH, GROUP * HEAD_DIM)]
            q = jnp.dot(x, w, preferred_element_type=F32) * Q_SCALE
            q = [q[:, h * HEAD_DIM:(h + 1) * HEAD_DIM] for h in range(GROUP)]
            return {A_UNIT: jnp.concatenate(q, axis=0).astype(BF16)}

        def scores(u):
            val["s", u] = lax.dot_general(val["q"][u], kv[slot, K, u], (((1,), (1,)), ((), ())),
                                          preferred_element_type=F32)

        def softmax(u):
            s = val["s", u]
            p = jnp.exp2(s - jnp.max(s, axis=-1, keepdims=True))
            val["inv", u] = 1.0 / jnp.sum(p, axis=-1, keepdims=True)
            val["p", u] = p.astype(BF16)

        def pv(u, r0, r1):
            return jnp.dot(val["p", u][:, r0:r1], kv[slot, V, u, pl.ds(r0, r1 - r0), :],
                           preferred_element_type=F32)

        def values(u):
            val["o", u] = pv(u, 0, SEQ_K) * val["inv", u]

        def values_head(u):
            partial[u] = pv(u, 0, V_SPLIT)

        def values_tail(u):
            val["o", u] = (partial[u] + pv(u, V_SPLIT, SEQ_K)) * val["inv", u]

        def project(heads, w, acc, b, col):
            rows = _ds(b, SEQ_Q)
            o = jnp.concatenate(heads, axis=1).astype(BF16)
            res = acc[rows, :] + jnp.dot(o, w, preferred_element_type=F32)
            acc[rows, :] = res
            out[b, :, pl.ds(col, D_MODEL)] = res.astype(BF16)

        def out_a():
            o = val["o", A_UNIT]
            project([o[h * SEQ_Q:(h + 1) * SEQ_Q] for h in range(GROUP)],
                    woa[_ds(unit // BATCH, GROUP * HEAD_DIM), :], acca, unit % BATCH, 0)

        def out_b():
            w = jnp.concatenate(
                [wob[_ds(_b_head(group, u), HEAD_DIM), :] for u in range(GROUP)], axis=0)
            project([val["o", u] for u in range(GROUP)], w, accb, group % BATCH, D_MODEL)

        table = {
            "qa": lambda: val["q"].update(q_a()),
            "qb": lambda: val["q"].update(q_b(group)),
            "qnext": lambda: val["qnext"].update(q_b(group + 1)),
            "oa": out_a,
            "ob": out_b,
        }
        for u in range(GROUP + 1):
            table[f"k{u}"] = lambda u=u: scores(u)
            table[f"s{u}"] = lambda u=u: softmax(u)
            table[f"v{u}"] = lambda u=u: values(u)
            table[f"head{u}"] = lambda u=u: values_head(u)
            table[f"tail{u}"] = lambda u=u: values_tail(u)
        return [table[name] for name in order.split()]

    def run(order, unit, group, slot, val):
        for stage in stages(order, unit, group, slot, val):
            stage()

    def row_page(src, dst, n, sem):
        return pltpu.make_async_copy(src.at[_ds(n, W_ROWS)], dst.at[_ds(n, W_ROWS)], w_sem.at[sem])

    def wq_page(src, dst, n, sem):
        idx = (_ds(n // 2, 8), _ds(n % 2, HEADS * HEAD_DIM // 2))
        return pltpu.make_async_copy(src.at[idx], dst.at[idx], w_sem.at[sem])

    def a_pages(kind, s):
        return [page(kind, s, s, n) for n in range(SET_PAGES) if PAGE_ORDER[kind][n][0] == A_UNIT]

    def stream(kind, first, last):
        return [page(kind, p // SET_PAGES, p // SET_PAGES % SLOTS, p % SET_PAGES)
                for p in range(first, last)]

    for n in range(BATCH * SEQ_Q // W_ROWS):
        row_page(xa_hbm, xa, n, 4).start(priority=1)
        row_page(xb_hbm, xb, n, 5).start(priority=1)
    for copy in a_pages(V, 0):
        copy.start(priority=1)

    @pl.loop(0, W_STEPS)
    def _(t):
        for n in [region * W_STEPS + t for region in range(W_REGIONS)]:
            start_pairs([row_page(woa_hbm, woa, n, 2), wq_page(wqa_hbm, wqa, n, 0)],
                        [row_page(wob_hbm, wob, n, 3), wq_page(wqb_hbm, wqb, n, 1)])

    base = AHEAD * SET_PAGES
    start_pairs(stream(V, base, base + V_LOOK),
                a_pages(K, 0) + a_pages(K, 1) + a_pages(V, 1) + stream(K, base, base + K_LOOK))
    acca[...] = jnp.zeros_like(acca)
    accb[...] = jnp.zeros_like(accb)
    for n, buf in enumerate((wqa, wqb, woa, wob, xa, xb)):
        wait_all(buf, w_sem.at[n])
    wait_a(0)
    run(HEAD_ORDER, 0, None, 0, {"q": {}})
    wait_a(1)
    start_pairs(stream(V, base + V_LOOK, base + V_LOOK + SET_PAGES),
                stream(K, base + K_LOOK, base + K_LOOK + SET_PAGES))
    run(HEAD_ORDER, 1, None, 1, {"q": {}})
    wait_a(AHEAD)
    for part in (KB, VB_HEAD, VB_TAIL):
        wait_b(AHEAD, part)

    @pl.loop(AHEAD, STEPS)
    def _(i):
        def start(kind, n):
            skip, n = divmod(LOOK[kind] + n, SET_PAGES)
            s = i + 1 + skip
            end = STEPS if PAGE_ORDER[kind][n][0] == A_UNIT else LAST_SET + 1
            issue = lambda: page(kind, s, s % SLOTS, n).start(priority=PRIORITY[kind])
            if STEPS + skip < end:
                issue()
            else:
                pl.when(s < end)(issue)

        def start_pair(n):
            start(V, n)
            start(K, n)

        work = stages(MAIN_ORDER, i, i - AHEAD, i % SLOTS, {"q": {}})
        _interleave(work, [lambda n=n: start_pair(n) for n in range(IN_COMPUTE)], 2, len(work))

        @pl.when(i >= AHEAD)
        def _():
            for n in range(IN_COMPUTE, SET_PAGES):
                start_pair(n)

        slot = (i + 1) % SLOTS
        pl.when(i + 1 < STEPS)(lambda: wait_a(slot))
        for part in (KB, VB_HEAD, VB_TAIL):
            wait_b(slot, part)

    slot = LAST_SET % SLOTS
    b_pages = lambda kind: [n for n in range(SET_PAGES) if PAGE_ORDER[kind][n][0] != A_UNIT]
    val = {"q": {}, "qnext": {}}
    _interleave(stages(TAIL_ORDER, None, STEPS - 2, (LAST_SET - 1) % SLOTS, val),
                [lambda n=n: page(K, LAST_SET, slot, n).start(priority=PRIORITY[K])
                 for n in b_pages(K) if n >= K_LOOK], 0, 8)
    val = {"q": val["qnext"]}
    wait_b(slot, KB)
    run("k0 k1 s0 k2 s1 k3 s2 s3", None, STEPS - 1, slot, val)
    wait_b(slot, VB_HEAD)

    def out_copy(b0, b1):
        rows = pl.ds(b0, b1 - b0)
        return pltpu.make_async_copy(out.at[rows], out_hbm.at[rows], out_sem)

    last_pages = [n for n in b_pages(V) if PAGE_ORDER[V][n][1] * PAGE >= V_SPLIT]
    for m, n in enumerate(last_pages):
        if m == WRITE_AT[0]:
            out_copy(0, EARLY_BATCHES).start()
            run("head0 head1 head2 head3", None, STEPS - 1, slot, val)
        if m == WRITE_AT[1]:
            out_copy(EARLY_BATCHES, BATCH - 1).start()
        page(V, LAST_SET, slot, n).wait()
    run("tail0 tail1 tail2 tail3 ob", None, STEPS - 1, slot, val)
    out_copy(BATCH - 1, BATCH).start()
    wait_all(out, out_sem)


@jax.jit
def pallas_concat_heads__gqa_block_cached__mha_block_cached__near_ridge_kernel(
    A_x: jax.Array,
    A_k_cache: jax.Array,
    A_v_cache: jax.Array,
    A_wq: jax.Array,
    A_wo: jax.Array,
    B_x: jax.Array,
    B_k_cache: jax.Array,
    B_v_cache: jax.Array,
    B_wq: jax.Array,
    B_wo: jax.Array,
):
    rows, inner = BATCH * SEQ_Q, HEADS * HEAD_DIM
    in_hbm = pl.BlockSpec(memory_space=pl.ANY)
    return pl.pallas_call(
        _kernel,
        in_specs=[in_hbm] * 10,
        out_specs=in_hbm,
        out_shape=jax.ShapeDtypeStruct((BATCH, SEQ_Q, 2 * D_MODEL), BF16),
        scratch_shapes=[
            pltpu.VMEM((rows, D_MODEL), BF16),
            pltpu.VMEM((rows, D_MODEL), BF16),
            pltpu.VMEM((D_MODEL, inner), BF16),
            pltpu.VMEM((D_MODEL, inner), BF16),
            pltpu.VMEM((inner, D_MODEL), BF16),
            pltpu.VMEM((inner, D_MODEL), BF16),
            pltpu.VMEM((SLOTS, 2, GROUP + 1, SEQ_K, HEAD_DIM), BF16),
            pltpu.VMEM((rows, D_MODEL), F32),
            pltpu.VMEM((rows, D_MODEL), F32),
            pltpu.VMEM((GROUP, SEQ_Q, HEAD_DIM), F32),
            pltpu.VMEM((BATCH, SEQ_Q, 2 * D_MODEL), BF16),
            pltpu.SemaphoreType.DMA((5 * SLOTS,)),
            pltpu.SemaphoreType.DMA((6,)),
            pltpu.SemaphoreType.DMA(()),
        ],
        compiler_params=pltpu.CompilerParams(
            vmem_limit_bytes=64 * 1024 * 1024,
            disable_bounds_checks=True,
            disable_semaphore_checks=True,
        ),
        name="fused_attn",
    )(A_x.reshape(rows, D_MODEL), A_k_cache, A_v_cache, A_wq, A_wo,
      B_x.reshape(rows, D_MODEL), B_k_cache, B_v_cache, B_wq, B_wo)
```
